```python
import os as _os
_os.environ.setdefault("JAX_PLATFORMS", "cpu")
import jax
import jax.numpy as jnp

def _softmax(x, axis=-1):
    return jax.nn.softmax(x, axis=axis)
def _gelu(x):
    return jax.nn.gelu(x, approximate=True)
def _silu(x):
    return jax.nn.silu(x)
def _sigmoid(x):
    return jax.nn.sigmoid(x)
def _layernorm(x, axis=-1, eps=1e-5):
    m = jnp.mean(x, axis=axis, keepdims=True)
    v = jnp.var(x, axis=axis, keepdims=True)
    return (x - m) / jnp.sqrt(v + eps)
def _scatter_add(tgt, idx, src, axis=0):
    return tgt.at[idx].add(src)
def _segment_sum(src, seg, n):
    return jax.ops.segment_sum(src, seg, n)
class _Rng:
    def __init__(self, key):
        self._k = key
    def _next(self):
        self._k, sub = jax.random.split(self._k)
        return sub
    def normal(self, shape):
        return jax.random.normal(self._next(), shape, dtype=jnp.bfloat16)
    def randint(self, lo, hi, shape):
        return jax.random.randint(self._next(), shape, lo, hi, dtype=jnp.int32)
    def uniform(self, shape, lo=0.0, hi=1.0):
        return jax.random.uniform(self._next(), shape, jnp.bfloat16, lo, hi)
    def permutation(self, n):
        return jax.random.permutation(self._next(), n)


kernel_name = 'standalone__mha_softmax__near_ridge'

def setup_inputs():
    _rng = _Rng(jax.random.key(int.from_bytes(__import__("os").urandom(4), "little")))
    _w = (lambda a: (lambda t: t.astype(jnp.bfloat16) if jnp.issubdtype(t.dtype, jnp.floating) else t)(jnp.asarray(a)))
    B, H, Sq, Sk, D = 8, 32, 496, 512, 192
    return {
        "q": _w((lambda *s: _rng.normal(s) * 0.05)(B, H, Sq, D)),
        "k": _w((lambda *s: _rng.normal(s) * 3.2)(B, H, Sk, D)),
        "v": _w((lambda *s: _rng.normal(s) * 0.05)(B, H, Sk, D)),
    }

def reference(q, k, v):
    scale = q.shape[-1] ** -0.5
    scores = jnp.einsum("bhqd,bhkd->bhqk", q, k) * scale
    p = _softmax(scores, axis=-1)
    return jnp.einsum("bhqk,bhkd->bhqd", p, v)
```

```python
import functools

import jax
import jax.numpy as jnp
import jax.experimental.pallas as pl
import jax.experimental.pallas.tpu as pltpu
import numpy as np

_LOG2E = float(np.log2(np.e))
_HB = 8


def _kernel(q_ref, k_ref, v_ref, o_ref, *, scale):
    c = scale * _LOG2E

    def qk(h):
        return jnp.dot(k_ref[0, h].T, q_ref[0, h], preferred_element_type=jnp.float32)

    def sm(sT):
        m = jnp.max(sT, axis=0, keepdims=True)
        p = jnp.exp2((sT - m) * c)
        l = jnp.sum(p, axis=0, keepdims=True)
        return p.astype(jnp.bfloat16), l

    def pv(h, p, l):
        oT = jnp.dot(v_ref[0, h], p, preferred_element_type=jnp.float32)
        o_ref[0, h] = (oT / l).astype(o_ref.dtype)

    S, P = {}, {}
    for i in range(_HB + 2):
        if i < _HB:
            S[i] = qk(i)
        if 0 <= i - 1 < _HB:
            P[i - 1] = sm(S.pop(i - 1))
        if 0 <= i - 2 < _HB:
            pv(i - 2, *P.pop(i - 2))


@jax.jit
def pallas_standalone__mha_softmax__near_ridge_kernel(q, k, v):
    B, H, Sq, D = q.shape
    Sk = k.shape[2]
    qT = jnp.swapaxes(q, 2, 3)
    kT = jnp.swapaxes(k, 2, 3)
    vT = jnp.swapaxes(v, 2, 3)
    oT = pl.pallas_call(
        functools.partial(_kernel, scale=D ** -0.5),
        grid=(B, H // _HB),
        in_specs=[
            pl.BlockSpec((1, _HB, D, Sq), lambda b, h: (b, h, 0, 0)),
            pl.BlockSpec((1, _HB, D, Sk), lambda b, h: (b, h, 0, 0)),
            pl.BlockSpec((1, _HB, D, Sk), lambda b, h: (b, h, 0, 0)),
        ],
        out_specs=pl.BlockSpec((1, _HB, D, Sq), lambda b, h: (b, h, 0, 0)),
        out_shape=jax.ShapeDtypeStruct((B, H, D, Sq), q.dtype),
        compiler_params=pltpu.CompilerParams(
            dimension_semantics=("parallel", "parallel"),
            vmem_limit_bytes=100 * 1024 * 1024,
            flags={"XLA_TPU_FORCE_LP_LLO_SCHEDULER": True},
        ),
    )(qT, kT, vT)
    return jnp.swapaxes(oT, 2, 3)
```

```python
import functools

import jax
import jax.numpy as jnp
from jax import lax
import jax.experimental.pallas as pl
import jax.experimental.pallas.tpu as pltpu
import numpy as np

_LOG2E = float(np.log2(np.e))

_U = 16
_GROUPS = (1, 1, 2, 2, 4, 6)
_NB = 2
_LAG_SM, _LAG_PV = 1, 2
_LANES = 128

_GOFF = tuple(sum(_GROUPS[:g]) for g in range(len(_GROUPS)))
_ARR = {"q": 0, "k": 1, "v": 2}


def _need_order():
    order = [("k", 0)]
    pend = {(a, g) for a in _ARR for g in range(len(_GROUPS))} - set(order)

    def need(a, u):
        for g in range(len(_GROUPS)):
            if _GOFF[g] <= u and (a, g) in pend:
                pend.discard((a, g))
                order.append((a, g))

    for i in range(_U + _LAG_PV):
        if i < _U:
            need("q", i)
            if i > 0:
                need("k", i)
        if 0 <= i - _LAG_PV < _U:
            need("v", i - _LAG_PV)
    assert not pend
    return tuple(order)


def _kernel(q_hbm, k_hbm, v_hbm, o_hbm, qb, kb, vb, ob, kt_scr, sems, osems, *, scale):
    n_heads = q_hbm.shape[0]
    d, sq = qb.shape[2], qb.shape[3]
    sq_pad = pl.cdiv(sq, _LANES) * _LANES
    n_iter = n_heads // _U
    c = scale * _LOG2E
    hbm = {"q": q_hbm, "k": k_hbm, "v": v_hbm}
    buf = {"q": qb, "k": kb, "v": vb}
    need_order = _need_order()

    def scaled_k(kT):
        return (kT.astype(jnp.float32) * c).astype(jnp.bfloat16).T

    def in_copy(a, h0, slot, g):
        off, n = _GOFF[g], _GROUPS[g]
        return pltpu.make_async_copy(
            hbm[a].at[pl.ds(h0 + off, n)], buf[a].at[slot, pl.ds(off, n)],
            sems.at[_ARR[a], slot, g])

    def start_block(h0, slot):
        for a, g in need_order:
            in_copy(a, h0, slot, g).start()

    def wait_out(slot):
        pltpu.make_async_copy(ob.at[slot], o_hbm.at[pl.ds(0, _U)], osems.at[slot]).wait()

    def body(j, carry):
        slot = j & 1
        h0 = j * _U
        waits = {(a, g) for a in _ARR for g in range(len(_GROUPS))} - {("k", 0)}
        deferred_out = []

        def need(a, u):
            for g in range(len(_GROUPS)):
                if _GOFF[g] <= u and (a, g) in waits:
                    waits.discard((a, g))
                    in_copy(a, 0, slot, g).wait()
            if not waits:
                for start in deferred_out:
                    start()
                deferred_out.clear()

        def qk(u):
            need("q", u)
            if u > 0:
                need("k", u)
            qT = qb[slot, u]
            qT = jnp.concatenate([qT, jnp.zeros((d, sq_pad - sq), qT.dtype)], axis=1)
            k = kt_scr[...] if u == 0 else scaled_k(kb[slot, u])
            sT = jnp.dot(k, qT, preferred_element_type=jnp.float32)
            if u == 2:
                start_block(jnp.minimum(h0 + _U, n_heads - _U), 1 - slot)
                pl.when(j >= _NB)(lambda: wait_out(slot))
            return sT

        def softmax(sT):
            m = jnp.max(sT, axis=0, keepdims=True)
            p = jnp.exp2(sT - m)
            l = jnp.sum(p, axis=0, keepdims=True)
            return p.astype(jnp.bfloat16), l

        def pv(u, p, l):
            need("v", u)
            oT = jnp.dot(vb[slot, u], p, preferred_element_type=jnp.float32)
            ob[slot, u] = (oT / l).astype(ob.dtype)[:, :sq]
            start = pltpu.make_async_copy(
                ob.at[slot, u], o_hbm.at[h0 + u], osems.at[slot]).start
            if waits:
                deferred_out.append(start)
            else:
                start()

        scores, probs = {}, {}
        for i in range(_U + _LAG_PV):
            if i < _U:
                scores[i] = qk(i)
            if 0 <= i - _LAG_SM < _U:
                probs[i - _LAG_SM] = softmax(scores.pop(i - _LAG_SM))
            if 0 <= i - _LAG_PV < _U:
                pv(i - _LAG_PV, *probs.pop(i - _LAG_PV))
            if i == _U - 1:
                in_copy("k", 0, 1 - slot, 0).wait()
                kt_scr[...] = scaled_k(kb[1 - slot, 0])
        assert not waits and not deferred_out
        return carry

    start_block(0, 0)
    in_copy("k", 0, 0, 0).wait()
    kt_scr[...] = scaled_k(kb[0, 0])
    lax.fori_loop(0, n_iter, body, 0)
    for a, g in need_order:
        if (a, g) != ("k", 0):
            in_copy(a, 0, n_iter % _NB, g).wait()
    for j in range(n_iter - _NB, n_iter):
        wait_out(j % _NB)


@jax.jit
def pallas_standalone__mha_softmax__near_ridge_kernel(q, k, v):
    B, H, Sq, D = q.shape
    Sk = k.shape[2]
    n_heads = B * H
    assert n_heads % _U == 0 and n_heads // _U >= _NB
    qT = jnp.swapaxes(q, 2, 3).reshape(n_heads, D, Sq)
    kT = jnp.swapaxes(k, 2, 3).reshape(n_heads, D, Sk)
    vT = jnp.swapaxes(v, 2, 3).reshape(n_heads, D, Sk)
    oT = pl.pallas_call(
        functools.partial(_kernel, scale=D ** -0.5),
        in_specs=[pl.BlockSpec(memory_space=pl.ANY)] * 3,
        out_specs=pl.BlockSpec(memory_space=pl.ANY),
        out_shape=jax.ShapeDtypeStruct((n_heads, D, Sq), q.dtype),
        scratch_shapes=[
            pltpu.VMEM((_NB, _U, D, Sq), q.dtype),
            pltpu.VMEM((_NB, _U, D, Sk), k.dtype),
            pltpu.VMEM((_NB, _U, D, Sk), v.dtype),
            pltpu.VMEM((_NB, _U, D, Sq), q.dtype),
            pltpu.VMEM((Sk, D), jnp.bfloat16),
            pltpu.SemaphoreType.DMA((3, _NB, len(_GROUPS))),
            pltpu.SemaphoreType.DMA((_NB,)),
        ],
        compiler_params=pltpu.CompilerParams(
            vmem_limit_bytes=100 * 1024 * 1024,
            disable_bounds_checks=True,
            flags={
                "XLA_TPU_FORCE_LP_LLO_SCHEDULER": True,
                "XLA_TPU_RESCHEDULE_DMA_DONES": True,
                "XLA_TPU_EVENLY_DISTRIBUTE_CRITICAL_NODES": True,
            },
        ),
    )(qT, kT, vT)
    return jnp.swapaxes(oT.reshape(B, H, D, Sq), 2, 3)
```
